```python
import os as _os
_os.environ.setdefault("JAX_PLATFORMS", "cpu")
import jax
import jax.numpy as jnp

def _softmax(x, axis=-1):
    return jax.nn.softmax(x, axis=axis)
def _gelu(x):
    return jax.nn.gelu(x, approximate=True)
def _silu(x):
    return jax.nn.silu(x)
def _sigmoid(x):
    return jax.nn.sigmoid(x)
def _layernorm(x, axis=-1, eps=1e-5):
    m = jnp.mean(x, axis=axis, keepdims=True)
    v = jnp.var(x, axis=axis, keepdims=True)
    return (x - m) / jnp.sqrt(v + eps)
def _scatter_add(tgt, idx, src, axis=0):
    return tgt.at[idx].add(src)
def _segment_sum(src, seg, n):
    return jax.ops.segment_sum(src, seg, n)
class _Rng:
    def __init__(self, key):
        self._k = key
    def _next(self):
        self._k, sub = jax.random.split(self._k)
        return sub
    def normal(self, shape):
        return jax.random.normal(self._next(), shape, dtype=jnp.bfloat16)
    def randint(self, lo, hi, shape):
        return jax.random.randint(self._next(), shape, lo, hi, dtype=jnp.int32)
    def uniform(self, shape, lo=0.0, hi=1.0):
        return jax.random.uniform(self._next(), shape, jnp.bfloat16, lo, hi)
    def permutation(self, n):
        return jax.random.permutation(self._next(), n)


kernel_name = 'sequential_preLN__linear_attn_block__dense_activation_squared_relu__prompt'

def setup_inputs():
    _rng = _Rng(jax.random.key(int.from_bytes(__import__("os").urandom(4), "little")))
    _w = (lambda a: (lambda t: t.astype(jnp.bfloat16) if jnp.issubdtype(t.dtype, jnp.floating) else t)(jnp.asarray(a)))
    def _A_setup():
        B, S, D = 1, 2048, 576
        return {
            "x": _w((lambda *s: _rng.normal(s) * 0.05)(B, S, D)),
            "wqkv": _w((lambda *s: _rng.normal(s) * 0.1)(D, 3 * D)),
            "wo": _w((lambda *s: _rng.normal(s) * 0.05)(D, D)),
        }
    _A_in = _A_setup()

    def _B_setup():
        B, S, D, F = 1, 2048, 576, 4608
        return {
            "x": _w((lambda *s: _rng.normal(s) * 0.05)(B, S, D)),
            "w1": _w((lambda *s: _rng.normal(s) * 0.05)(D, F)),
            "b1": _w((lambda *s: _rng.normal(s) * 0.05)(F)),
            "w2": _w((lambda *s: _rng.normal(s) * 0.05)(F, D)),
            "b2": _w((lambda *s: _rng.normal(s) * 0.05)(D)),
        }
    _B_in = _B_setup()

    return {
        "A_x": _A_in["x"],
        "A_wqkv": _A_in["wqkv"],
        "A_wo": _A_in["wo"],
        "B_x": _B_in["x"],
        "B_w1": _B_in["w1"],
        "B_b1": _B_in["b1"],
        "B_w2": _B_in["w2"],
        "B_b2": _B_in["b2"],
    }

def reference(A_x, A_wqkv, A_wo, B_x, B_w1, B_b1, B_w2, B_b2):
    def _A_ref(x, wqkv, wo):
        B, S, D = x.shape
        H = 32; Dh = D // H
        qkv = (lambda x, *d: x.transpose(*d))((x @ wqkv).reshape(B, S, 3, H, Dh), 2, 0, 3, 1, 4)
        q, k, v = qkv[0], qkv[1], qkv[2]
        phi = lambda t: jnp.where(t > 0, t + 1, jnp.exp(t)) + 1e-6
        pq, pk = phi(q), phi(k)
        kv = jnp.einsum("bhsd,bhse->bhde", pk, v)
        z = jnp.einsum("bhsd->bhd", pk)
        num = jnp.einsum("bhqd,bhde->bhqe", pq, kv)
        den = jnp.einsum("bhqd,bhd->bhq", pq, z)[..., None] + 1e-6
        o = num / den
        return (lambda x, *d: x.transpose(*d))(o, 0, 2, 1, 3).reshape(B, S, D) @ wo

    def _B_ref(x, w1, b1, w2, b2):
        h = jnp.einsum("bsd,df->bsf", x, w1) + b1
        zero = jnp.zeros_like(h)
        r = jnp.where(h > zero, h, zero)
        h = r * r
        out = jnp.einsum("bsf,fd->bsd", h, w2) + b2
        return out

    x = A_x
    h = x + _A_ref(_layernorm(x, axis=-1), A_wqkv, A_wo)
    h2 = h + _B_ref(_layernorm(h, axis=-1), B_w1, B_b1, B_w2, B_b2)
    return h2
```

```python
import functools
import jax
import jax.numpy as jnp
from jax import lax
import jax.experimental.pallas as pl
import jax.experimental.pallas.tpu as pltpu

S, D, H, DH, F = 2048, 576, 32, 18, 4608
DP = 640
QKV = 3 * D
EPS_LN = 1e-5
GH = 4
GR = GH * DH
NG = H // GH
GA = GR + 8
QCH = ((512, 1152), (1152, 1728), (0, 512))
TM = 512
NT = S // TM


def _ln_t(x):
    m = jnp.mean(x, axis=0, keepdims=True)
    xc = x - m
    v = jnp.mean(xc * xc, axis=0, keepdims=True)
    return xc * lax.rsqrt(v + EPS_LN)


def _phi(t):
    return jnp.where(t > 0, t + 1.0, jnp.exp(t)) + 1e-6


def _mm(a, b):
    return jnp.dot(a, b, preferred_element_type=jnp.float32)


def make_kernel(fc, sub0, kpos):
    tm = TM
    nF = F // fc
    w1_chunks = 3
    wc = F // w1_chunks
    nS0 = tm // sub0

    def kernel(b1_hbm, b2_hbm, xt_hbm, wqkv_hbm, wo_hbm, w1_hbm, w2t_hbm, out_hbm,
               xt_s, wqa_s, wqb_s, wqc_s, wat_s, wvt_s, wqt_s, wo_s, w1_s, w1t_s, w2t_s,
               kv_s, maug_s, mt_s, e_s, b2c_s, b1_ref, b2_ref,
               out0_s, out1_s, out2_s, out3_s,
               sem_x0, sem_x, sem_q, sem_w, sem_w1, sem_o):
        outs = (out0_s, out1_s, out2_s, out3_s)
        wq_raw = (wqa_s, wqb_s, wqc_s)

        def tsl(t):
            return slice(t * tm, (t + 1) * tm)

        def x0_copy(s):
            return pltpu.make_async_copy(xt_hbm.at[:, s * sub0:(s + 1) * sub0],
                                         xt_s.at[:, s * sub0:(s + 1) * sub0], sem_x0.at[s])

        def x_copy(t):
            return pltpu.make_async_copy(xt_hbm.at[:, tsl(t)], xt_s.at[:, tsl(t)],
                                         sem_x.at[t])

        def w1_copy(c):
            return pltpu.make_async_copy(w1_hbm.at[:, c * wc:(c + 1) * wc],
                                         w1_s.at[0:D, c * wc:(c + 1) * wc], sem_w1.at[c])

        def q_copy(c):
            lo, hi = QCH[c]
            return pltpu.make_async_copy(wqkv_hbm.at[:, lo:hi], wq_raw[c], sem_q.at[c])

        wo_copy = pltpu.make_async_copy(wo_hbm, wo_s, sem_w.at[0])
        w2_copy = pltpu.make_async_copy(w2t_hbm, w2t_s, sem_w.at[1])
        b1_copy = pltpu.make_async_copy(b1_hbm, b1_ref, sem_w.at[2])
        b2_copy = pltpu.make_async_copy(b2_hbm, b2_ref, sem_w.at[3])

        q_copy(0).start()
        for s in range(nS0):
            x0_copy(s).start()
        q_copy(1).start()
        x_copy(1).start()
        b1_copy.start()
        b2_copy.start()

        r3 = lax.broadcasted_iota(jnp.int32, (D, 2 * H), 0) // DH
        c3 = lax.broadcasted_iota(jnp.int32, (D, 2 * H), 1)
        e_s[...] = jnp.where((r3 == c3) | (r3 == c3 - H), 1.0, 0.0).astype(jnp.bfloat16)

        def bias_setup():
            b2b = jnp.broadcast_to(b2_ref[...].astype(jnp.float32).reshape(1, D), (128, D))
            b2c_s[...] = b2b.T
            rr = lax.broadcasted_iota(jnp.int32, (DP - D, F), 0)
            b1f = jnp.broadcast_to(b1_ref[...].astype(jnp.float32).reshape(1, F), (DP - D, F))
            w1_s[D:DP, :] = jnp.where(rr == 0, b1f, 0.0).astype(jnp.bfloat16)

        def transpose_w1(c):
            w = 512
            for cc in range(wc // w):
                lo = c * wc + cc * w
                w1t_s[lo:lo + w, :] = w1_s[:, lo:lo + w].T

        def ln1(t):
            return _ln_t(xt_s[:, tsl(t)].astype(jnp.float32)).astype(jnp.bfloat16)

        def kproj(xn):
            return _mm(wat_s[64:64 + D, :], xn)

        def vproj(xn):
            return _mm(wvt_s[...], xn)

        def kv_accum(t, k, v):
            ones = jnp.ones((GA - GR, tm), jnp.float32)
            for g in range(NG):
                pk = _phi(k[g * GR:(g + 1) * GR]).astype(jnp.bfloat16)
                va = jnp.concatenate([v[g * GR:(g + 1) * GR], ones],
                                     axis=0).astype(jnp.bfloat16)
                kvg = lax.dot_general(pk, va, (((1,), (1,)), ((), ())),
                                      preferred_element_type=jnp.float32)
                if t == 0:
                    kv_s[g] = kvg
                else:
                    kv_s[g] += kvg

        def qproj(xn):
            return _phi(_mm(wqt_s[...], xn)).astype(jnp.bfloat16)

        def den_step(pq):
            den = _mm(mt_s[D:DP, :], pq) + 1e-6
            inv = 1.0 / den
            hi = inv.astype(jnp.bfloat16).astype(jnp.float32)
            row = lax.broadcasted_iota(jnp.int32, (2 * H, tm), 0)
            return jnp.where(row < H, hi, inv - hi).astype(jnp.bfloat16)

        def bc_step(pq, hl):
            invb = _mm(e_s[...], hl)
            return (pq.astype(jnp.float32) * invb).astype(jnp.bfloat16)

        def attn_step(t, pqs):
            h = xt_s[:, tsl(t)].astype(jnp.float32) + _mm(mt_s[0:D, :], pqs)
            hn = _ln_t(h).astype(jnp.bfloat16)
            rr2 = lax.broadcasted_iota(jnp.int32, (DP - D, tm), 0)
            aug = jnp.where(rr2 == 0, 1.0, 0.0).astype(jnp.bfloat16)
            return jnp.concatenate([hn, aug], axis=0), h + b2c_s[:, 0:1]

        q_copy(0).wait()
        for s in range(nS0):
            x0_copy(s).wait()
        wat_s[...] = wqa_s[...].T
        xn0 = ln1(0)
        x_copy(2).start()
        x_copy(3).start()
        q_copy(2).start()
        w1_copy(0).start()
        k0 = kproj(xn0)
        q_copy(1).wait()
        x_copy(1).wait()
        wvt_s[...] = wqb_s[...].T
        xn1 = ln1(1)
        v0 = vproj(xn0)
        k1 = kproj(xn1)
        x_copy(2).wait()
        x_copy(3).wait()
        q_copy(2).wait()
        w1_copy(0).wait()
        b1_copy.wait()
        b2_copy.wait()
        w1_copy(1).start()
        w1_copy(2).start()
        wo_copy.start()
        v1 = vproj(xn1)
        bias_setup()
        xn2 = ln1(2)
        transpose_w1(0)
        kv_accum(0, k0, v0)
        k2 = kproj(xn2)
        wqt_s[0:512, :] = wqc_s[...].T
        wqt_s[512:D, :] = wat_s[0:64, :]
        xn3 = ln1(3)
        v2 = vproj(xn2)
        kv_accum(1, k1, v1)
        w1_copy(1).wait()
        w1_copy(2).wait()
        wo_copy.wait()
        w2_copy.start()
        k3 = kproj(xn3)
        transpose_w1(1)
        v3 = vproj(xn3)
        transpose_w1(2)
        kv_accum(2, k2, v2)
        pq0 = qproj(xn0)
        kv_accum(3, k3, v3)
        pq1 = qproj(xn1)

        wof = wo_s[...].astype(jnp.float32)
        rg = lax.broadcasted_iota(jnp.int32, (GR, GR), 0) // DH
        cg = lax.broadcasted_iota(jnp.int32, (GR, GR), 1) // DH
        rz = lax.broadcasted_iota(jnp.int32, (GR, 2 * H), 0) // DH
        cz = lax.broadcasted_iota(jnp.int32, (GR, 2 * H), 1)
        for g in range(NG):
            kvg = kv_s[g]
            kvm = jnp.where(rg == cg, kvg[:, 0:GR], 0.0).astype(jnp.bfloat16)
            wog = wof[g * GR:(g + 1) * GR].astype(jnp.bfloat16)
            maug_s[g * GR:(g + 1) * GR, 0:D] = _mm(kvm, wog)
            zcol = kvg[:, GR:GR + 1]
            hh = rz + g * GH
            maug_s[g * GR:(g + 1) * GR, D:DP] = jnp.where(
                (hh == cz) | (hh == cz - H), zcol, 0.0)
        mt_s[...] = maug_s[...].T.astype(jnp.bfloat16)
        pq2 = qproj(xn2)
        hl0 = den_step(pq0)
        hl1 = den_step(pq1)
        pqs0 = bc_step(pq0, hl0)
        pqs1 = bc_step(pq1, hl1)
        hh_ = [None] * NT
        hh_[0] = attn_step(0, pqs0)
        hh_[1] = attn_step(1, pqs1)
        w2_copy.wait()

        def out_copy(t):
            return pltpu.make_async_copy(outs[t], out_hbm.at[:, tsl(t)], sem_o.at[t])

        st = {}

        def extra(t, c):
            if t == 0:
                if c == kpos:
                    st['hl'] = den_step(pq2)
                elif c == kpos + 1:
                    st['pqs'] = bc_step(pq2, st['hl'])
                elif c == kpos + 2:
                    hh_[2] = attn_step(2, st['pqs'])
            elif t == 1:
                if c == kpos:
                    st['pq'] = qproj(xn3)
                elif c == kpos + 1:
                    st['hl'] = den_step(st['pq'])
                elif c == kpos + 2:
                    st['pqs'] = bc_step(st['pq'], st['hl'])
                elif c == kpos + 3:
                    hh_[3] = attn_step(3, st['pqs'])

        for t in range(NT):
            hna, acc = hh_[t]
            for c in range(nF):
                extra(t, c)
                h1 = _mm(w1t_s[c * fc:(c + 1) * fc, :], hna)
                r = jnp.maximum(h1, 0.0)
                act = (r * r).astype(jnp.bfloat16)
                acc = acc + _mm(w2t_s[:, c * fc:(c + 1) * fc], act)
            outs[t][...] = acc.astype(jnp.bfloat16)
            out_copy(t).start()

        for t in range(NT):
            out_copy(t).wait()

    return kernel, nS0, w1_chunks


def build(fc=512, vmem_mb=110, sub0=512, kpos=2):
    kernel, nS0, w1_chunks = make_kernel(fc, sub0, kpos)

    def fn(A_x, A_wqkv, A_wo, B_x, B_w1, B_b1, B_w2, B_b2):
        xt = A_x.reshape(S, D).T
        w2t = B_w2.T
        out = pl.pallas_call(
            kernel,
            in_specs=[pl.BlockSpec(memory_space=pl.ANY)] * 7,
            out_specs=pl.BlockSpec(memory_space=pl.ANY),
            out_shape=jax.ShapeDtypeStruct((D, S), jnp.bfloat16),
            scratch_shapes=[
                pltpu.VMEM((D, S), jnp.bfloat16),
                pltpu.VMEM((D, 640), jnp.bfloat16),
                pltpu.VMEM((D, 576), jnp.bfloat16),
                pltpu.VMEM((D, 512), jnp.bfloat16),
                pltpu.VMEM((640, D), jnp.bfloat16),
                pltpu.VMEM((D, D), jnp.bfloat16),
                pltpu.VMEM((D, D), jnp.bfloat16),
                pltpu.VMEM((D, D), jnp.bfloat16),
                pltpu.VMEM((DP, F), jnp.bfloat16),
                pltpu.VMEM((F, DP), jnp.bfloat16),
                pltpu.VMEM((D, F), jnp.bfloat16),
                pltpu.VMEM((NG, GR, GA), jnp.float32),
                pltpu.VMEM((D, DP), jnp.float32),
                pltpu.VMEM((DP, D), jnp.bfloat16),
                pltpu.VMEM((D, 2 * H), jnp.bfloat16),
                pltpu.VMEM((D, 128), jnp.float32),
                pltpu.VMEM((F,), jnp.bfloat16),
                pltpu.VMEM((D,), jnp.bfloat16),
                pltpu.VMEM((D, TM), jnp.bfloat16),
                pltpu.VMEM((D, TM), jnp.bfloat16),
                pltpu.VMEM((D, TM), jnp.bfloat16),
                pltpu.VMEM((D, TM), jnp.bfloat16),
                pltpu.SemaphoreType.DMA((nS0,)),
                pltpu.SemaphoreType.DMA((NT,)),
                pltpu.SemaphoreType.DMA((3,)),
                pltpu.SemaphoreType.DMA((4,)),
                pltpu.SemaphoreType.DMA((w1_chunks,)),
                pltpu.SemaphoreType.DMA((NT,)),
            ],
            compiler_params=pltpu.CompilerParams(
                vmem_limit_bytes=vmem_mb * 1024 * 1024),
        )(B_b1, B_b2, xt, A_wqkv, A_wo, B_w1, w2t)
        return out.T.reshape(1, S, D)

    return fn


pallas_sequential_preLN__linear_attn_block__dense_activation_squared_relu__prompt_kernel = jax.jit(build())
```

```python
import jax
import jax.numpy as jnp
from jax import lax
import jax.experimental.pallas as pl
import jax.experimental.pallas.tpu as pltpu

S, D, H, DH, F = 2048, 576, 32, 18, 4608
DP = 640
EPS_LN = 1e-5
GH = 4
GR = GH * DH
NG = H // GH
GA = GR + 8
QCH = ((512, 1152), (1152, 1728), (0, 512))
TM = 512
NT = S // TM
FC = 1536
NFC = F // FC
W1B = (0, 1024, 2560, 4608)


def _ln_t(x):
    m = jnp.mean(x, axis=0, keepdims=True)
    xc = x - m
    v = jnp.mean(xc * xc, axis=0, keepdims=True)
    return xc * lax.rsqrt(v + EPS_LN)


def _phi(t):
    return jnp.where(t > 0, t + 1.0, jnp.exp(t)) + 1e-6


def _mm(a, b):
    return jnp.dot(a, b, preferred_element_type=jnp.float32)


def _kernel(b1_hbm, b2_hbm, xt_hbm, wqkv_hbm, wo_hbm, w1_hbm, w2t_hbm, out_hbm,
            xt_s, wqa_s, wqb_s, wqc_s, wat_s, wvt_s, wqt_s, wo_s, w1_s, w1t_s, w2t_s,
            kv_s, maug_s, mt_s, b2c_s, b1_s, b2_s, hna_s, h_s, out_s,
            sem_x, sem_q, sem_w, sem_w1, sem_o):
    tm = TM
    wq_raw = (wqa_s, wqb_s, wqc_s)

    def tsl(t):
        return slice(t * tm, (t + 1) * tm)

    def x_copy(t):
        return pltpu.make_async_copy(xt_hbm.at[:, tsl(t)], xt_s.at[:, tsl(t)],
                                     sem_x.at[t])

    def w1_copy(c):
        return pltpu.make_async_copy(w1_hbm.at[:, W1B[c]:W1B[c + 1]],
                                     w1_s.at[0:D, W1B[c]:W1B[c + 1]], sem_w1.at[c])

    def q_copy(c):
        lo, hi = QCH[c]
        return pltpu.make_async_copy(wqkv_hbm.at[:, lo:hi], wq_raw[c], sem_q.at[c])

    wo_copy = pltpu.make_async_copy(wo_hbm, wo_s, sem_w.at[0])
    w2_copy = pltpu.make_async_copy(w2t_hbm, w2t_s, sem_w.at[1])
    b1_copy = pltpu.make_async_copy(b1_hbm, b1_s, sem_w.at[2])
    b2_copy = pltpu.make_async_copy(b2_hbm, b2_s, sem_w.at[3])

    q_copy(0).start()
    x_copy(0).start()
    q_copy(1).start()
    x_copy(1).start()
    b1_copy.start()
    b2_copy.start()

    def bias_setup():
        b2b = jnp.broadcast_to(b2_s[...].astype(jnp.float32).reshape(1, D), (128, D))
        b2c_s[...] = b2b.T
        rr = lax.broadcasted_iota(jnp.int32, (DP - D, F), 0)
        b1f = jnp.broadcast_to(b1_s[...].astype(jnp.float32).reshape(1, F), (DP - D, F))
        w1_s[D:DP, :] = jnp.where(rr == 0, b1f, 0.0).astype(jnp.bfloat16)

    def transpose_w1(c):
        for lo in range(W1B[c], W1B[c + 1], 512):
            w1t_s[lo:lo + 512, :] = w1_s[:, lo:lo + 512].T

    def ln1(t):
        return _ln_t(xt_s[:, tsl(t)].astype(jnp.float32)).astype(jnp.bfloat16)

    def kproj(xn):
        return _mm(wat_s[64:64 + D, :], xn)

    def vproj(xn):
        return _mm(wvt_s[...], xn)

    def kv_accum(t, k, v):
        ones = jnp.ones((GA - GR, tm), jnp.float32)
        for g in range(NG):
            pk = _phi(k[g * GR:(g + 1) * GR]).astype(jnp.bfloat16)
            va = jnp.concatenate([v[g * GR:(g + 1) * GR], ones],
                                 axis=0).astype(jnp.bfloat16)
            kvg = lax.dot_general(pk, va, (((1,), (1,)), ((), ())),
                                  preferred_element_type=jnp.float32)
            if t == 0:
                kv_s[g] = kvg
            else:
                kv_s[g] += kvg

    def qproj(xn):
        return _phi(_mm(wqt_s[...], xn)).astype(jnp.bfloat16)

    def norm_step(pq):
        inv = 1.0 / (_mm(mt_s[D:D + H, :], pq) + 1e-6)
        i8 = lax.broadcasted_iota(jnp.int32, (8, tm), 0)
        blocks = []
        for j in range(D // 8):
            r0 = 8 * j
            ha, hb = r0 // DH, (r0 + 7) // DH
            ba = jnp.broadcast_to(inv[ha:ha + 1], (8, tm))
            if ha == hb:
                blocks.append(ba)
            else:
                bb = jnp.broadcast_to(inv[hb:hb + 1], (8, tm))
                blocks.append(jnp.where(i8 < DH * hb - r0, ba, bb))
        invb = jnp.concatenate(blocks, axis=0)
        return (pq.astype(jnp.float32) * invb).astype(jnp.bfloat16)

    def attn_step(t, pqs):
        h = xt_s[:, tsl(t)].astype(jnp.float32) + _mm(mt_s[0:D, :], pqs)
        hn = _ln_t(h).astype(jnp.bfloat16)
        rr2 = lax.broadcasted_iota(jnp.int32, (DP - D, tm), 0)
        aug = jnp.where(rr2 == 0, 1.0, 0.0).astype(jnp.bfloat16)
        hna_s[t] = jnp.concatenate([hn, aug], axis=0)
        h_s[t] = h + b2c_s[:, 0:1]

    q_copy(0).wait()
    x_copy(0).wait()
    wat_s[...] = wqa_s[...].T
    xn0 = ln1(0)
    x_copy(2).start()
    x_copy(3).start()
    q_copy(2).start()
    w1_copy(0).start()
    k0 = kproj(xn0)
    q_copy(1).wait()
    x_copy(1).wait()
    wvt_s[...] = wqb_s[...].T
    xn1 = ln1(1)
    v0 = vproj(xn0)
    k1 = kproj(xn1)
    x_copy(2).wait()
    x_copy(3).wait()
    q_copy(2).wait()
    w1_copy(0).wait()
    b1_copy.wait()
    b2_copy.wait()
    w1_copy(1).start()
    w1_copy(2).start()
    wo_copy.start()
    v1 = vproj(xn1)
    bias_setup()
    xn2 = ln1(2)
    transpose_w1(0)
    kv_accum(0, k0, v0)
    k2 = kproj(xn2)
    wqt_s[0:512, :] = wqc_s[...].T
    wqt_s[512:D, :] = wat_s[0:64, :]
    xn3 = ln1(3)
    v2 = vproj(xn2)
    kv_accum(1, k1, v1)
    w1_copy(1).wait()
    w1_copy(2).wait()
    wo_copy.wait()
    w2_copy.start()
    k3 = kproj(xn3)
    transpose_w1(1)
    v3 = vproj(xn3)
    transpose_w1(2)
    kv_accum(2, k2, v2)
    pq0 = qproj(xn0)
    kv_accum(3, k3, v3)
    pq1 = qproj(xn1)

    wof = wo_s[...].astype(jnp.float32)
    rg = lax.broadcasted_iota(jnp.int32, (GR, GR), 0) // DH
    cg = lax.broadcasted_iota(jnp.int32, (GR, GR), 1) // DH
    rz = lax.broadcasted_iota(jnp.int32, (GR, DP - D), 0) // DH
    cz = lax.broadcasted_iota(jnp.int32, (GR, DP - D), 1)
    for g in range(NG):
        kvg = kv_s[g]
        kvm = jnp.where(rg == cg, kvg[:, 0:GR], 0.0).astype(jnp.bfloat16)
        wog = wof[g * GR:(g + 1) * GR].astype(jnp.bfloat16)
        maug_s[g * GR:(g + 1) * GR, 0:D] = _mm(kvm, wog)
        zcol = kvg[:, GR:GR + 1]
        maug_s[g * GR:(g + 1) * GR, D:DP] = jnp.where(rz + g * GH == cz, zcol, 0.0)
    mt_s[...] = maug_s[...].T.astype(jnp.bfloat16)

    pq2 = qproj(xn2)
    ps0 = norm_step(pq0)
    ps1 = norm_step(pq1)
    pq3 = qproj(xn3)
    ps2 = norm_step(pq2)
    attn_step(0, ps0)
    attn_step(1, ps1)
    ps3 = norm_step(pq3)
    attn_step(2, ps2)
    attn_step(3, ps3)
    w2_copy.wait()

    def out_copy(t):
        col0 = t * tm if isinstance(t, int) else pl.multiple_of(t * tm, tm)
        return pltpu.make_async_copy(out_s.at[t], out_hbm.at[:, pl.ds(col0, tm)],
                                     sem_o.at[t])

    def body(it, carry):
        t = it // NFC
        c = it % NFC
        off = pl.multiple_of(c * FC, FC)
        h1 = _mm(w1t_s[pl.ds(off, FC), :], hna_s[t])
        r = jnp.maximum(h1, 0.0)
        act = (r * r).astype(jnp.bfloat16)
        acc = h_s[t] + _mm(w2t_s[:, pl.ds(off, FC)], act)
        h_s[t] = acc

        @pl.when(c == NFC - 1)
        def _():
            out_s[t] = acc.astype(jnp.bfloat16)
            out_copy(t).start()

        return carry

    lax.fori_loop(0, NT * NFC, body, 0)
    for t in range(NT):
        out_copy(t).wait()


@jax.jit
def pallas_sequential_preLN__linear_attn_block__dense_activation_squared_relu__prompt_kernel(
    A_x: jax.Array,
    A_wqkv: jax.Array,
    A_wo: jax.Array,
    B_x: jax.Array,
    B_w1: jax.Array,
    B_b1: jax.Array,
    B_w2: jax.Array,
    B_b2: jax.Array,
):
    del B_x
    xt = A_x.reshape(S, D).T
    w2t = B_w2.T
    out = pl.pallas_call(
        _kernel,
        in_specs=[pl.BlockSpec(memory_space=pl.ANY)] * 7,
        out_specs=pl.BlockSpec(memory_space=pl.ANY),
        out_shape=jax.ShapeDtypeStruct((D, S), jnp.bfloat16),
        scratch_shapes=[
            pltpu.VMEM((D, S), jnp.bfloat16),
            pltpu.VMEM((D, 640), jnp.bfloat16),
            pltpu.VMEM((D, 576), jnp.bfloat16),
            pltpu.VMEM((D, 512), jnp.bfloat16),
            pltpu.VMEM((640, D), jnp.bfloat16),
            pltpu.VMEM((D, D), jnp.bfloat16),
            pltpu.VMEM((D, D), jnp.bfloat16),
            pltpu.VMEM((D, D), jnp.bfloat16),
            pltpu.VMEM((DP, F), jnp.bfloat16),
            pltpu.VMEM((F, DP), jnp.bfloat16),
            pltpu.VMEM((D, F), jnp.bfloat16),
            pltpu.VMEM((NG, GR, GA), jnp.float32),
            pltpu.VMEM((D, DP), jnp.float32),
            pltpu.VMEM((DP, D), jnp.bfloat16),
            pltpu.VMEM((D, 128), jnp.float32),
            pltpu.VMEM((F,), jnp.bfloat16),
            pltpu.VMEM((D,), jnp.bfloat16),
            pltpu.VMEM((NT, DP, TM), jnp.bfloat16),
            pltpu.VMEM((NT, D, TM), jnp.float32),
            pltpu.VMEM((NT, D, TM), jnp.bfloat16),
            pltpu.SemaphoreType.DMA((NT,)),
            pltpu.SemaphoreType.DMA((3,)),
            pltpu.SemaphoreType.DMA((4,)),
            pltpu.SemaphoreType.DMA((3,)),
            pltpu.SemaphoreType.DMA((NT,)),
        ],
        compiler_params=pltpu.CompilerParams(vmem_limit_bytes=110 * 1024 * 1024),
    )(B_b1, B_b2, xt, A_wqkv, A_wo, B_w1, w2t)
    return out.T.reshape(1, S, D)
```
